```python
import os as _os
_os.environ.setdefault("JAX_PLATFORMS", "cpu")
import jax
import jax.numpy as jnp

def _softmax(x, axis=-1):
    return jax.nn.softmax(x, axis=axis)
def _gelu(x):
    return jax.nn.gelu(x, approximate=True)
def _silu(x):
    return jax.nn.silu(x)
def _sigmoid(x):
    return jax.nn.sigmoid(x)
def _layernorm(x, axis=-1, eps=1e-5):
    m = jnp.mean(x, axis=axis, keepdims=True)
    v = jnp.var(x, axis=axis, keepdims=True)
    return (x - m) / jnp.sqrt(v + eps)
def _scatter_add(tgt, idx, src, axis=0):
    return tgt.at[idx].add(src)
def _segment_sum(src, seg, n):
    return jax.ops.segment_sum(src, seg, n)
class _Rng:
    def __init__(self, key):
        self._k = key
    def _next(self):
        self._k, sub = jax.random.split(self._k)
        return sub
    def normal(self, shape):
        return jax.random.normal(self._next(), shape, dtype=jnp.bfloat16)
    def randint(self, lo, hi, shape):
        return jax.random.randint(self._next(), shape, lo, hi, dtype=jnp.int32)
    def uniform(self, shape, lo=0.0, hi=1.0):
        return jax.random.uniform(self._next(), shape, jnp.bfloat16, lo, hi)
    def permutation(self, n):
        return jax.random.permutation(self._next(), n)


kernel_name = 'sequential_preLN__mha_block__dense_activation_mish__prompt'

def setup_inputs():
    _rng = _Rng(jax.random.key(int.from_bytes(__import__("os").urandom(4), "little")))
    _w = (lambda a: (lambda t: t.astype(jnp.bfloat16) if jnp.issubdtype(t.dtype, jnp.floating) else t)(jnp.asarray(a)))
    def _A_setup():
        B, S, D, H = 1, 2048, 576, 32
        return {
            "x": _w((lambda *s: _rng.normal(s) * 0.05)(B, S, D)),
            "wqkv": _w((lambda *s: _rng.normal(s) * 0.05)(D, 3 * D)),
            "wo": _w((lambda *s: _rng.normal(s) * 0.05)(D, D)),
        }
    _A_in = _A_setup()

    def _B_setup():
        B, S, D, F = 1, 2048, 576, 4608
        return {
            "x": _w((lambda *s: _rng.normal(s) * 0.05)(B, S, D)),
            "w1": _w((lambda *s: _rng.normal(s) * 1.6)(D, F) * (D ** -0.5)),
            "b1": _w((lambda *s: _rng.normal(s) * 0.05)(F)),
            "w2": _w((lambda *s: _rng.normal(s) * 0.05)(F, D) * (F ** -0.5)),
        }
    _B_in = _B_setup()

    return {
        "A_x": _A_in["x"],
        "A_wqkv": _A_in["wqkv"],
        "A_wo": _A_in["wo"],
        "B_x": _B_in["x"],
        "B_w1": _B_in["w1"],
        "B_b1": _B_in["b1"],
        "B_w2": _B_in["w2"],
    }

def reference(A_x, A_wqkv, A_wo, B_x, B_w1, B_b1, B_w2):
    def _A_ref(x, wqkv, wo):
        B, S, D = x.shape
        H = 32
        Dh = D // H
        qkv = (lambda x, *d: x.transpose(*d))((x @ wqkv).reshape(B, S, 3, H, Dh), 2, 0, 3, 1, 4)
        q, k, v = qkv[0], qkv[1], qkv[2]
        scores = jnp.einsum("bhqd,bhkd->bhqk", q, k) * (Dh ** -0.5)
        p = _softmax(scores, axis=-1)
        o = jnp.einsum("bhqk,bhkd->bhqd", p, v)
        return (lambda x, *d: x.transpose(*d))(o, 0, 2, 1, 3).reshape(B, S, D) @ wo

    def _B_ref(x, w1, b1, w2):
        h = jnp.einsum("bsd,df->bsf", x, w1) + b1
        sp = jnp.log1p(jnp.exp(-jnp.abs(h))) + jnp.where(h > 0, h, jnp.zeros_like(h))
        act = h * jnp.tanh(sp)
        return jnp.einsum("bsf,fd->bsd", act, w2)

    x = A_x
    h = x + _A_ref(_layernorm(x, axis=-1), A_wqkv, A_wo)
    h2 = h + _B_ref(_layernorm(h, axis=-1), B_w1, B_b1, B_w2)
    return h2
```

```python
import jax
import jax.numpy as jnp
import jax.experimental.pallas as pl
import jax.experimental.pallas.tpu as pltpu

_H = 32
_HPG = 7
_LANES = 128
_EPS = 1e-5
_LOG2E = 1.4426950408889634


def _layernorm(x):
    m = jnp.mean(x, axis=-1, keepdims=True)
    xc = x - m
    v = jnp.mean(xc * xc, axis=-1, keepdims=True)
    return xc * jax.lax.rsqrt(v + _EPS)


@jax.jit
def pallas_sequential_preLN__mha_block__dense_activation_mish__prompt_kernel(
    A_x: jax.Array,
    A_wqkv: jax.Array,
    A_wo: jax.Array,
    B_x: jax.Array,
    B_w1: jax.Array,
    B_b1: jax.Array,
    B_w2: jax.Array,
):
    B, S, D = A_x.shape
    assert B == 1
    F = B_w1.shape[1]
    dh = D // _H
    ng = -(-_H // _HPG)
    gw = [min(_HPG, _H - g * _HPG) * dh for g in range(ng)]
    TQ = 256
    NQ = S // TQ
    RC = 512
    scale = (dh ** -0.5) * _LOG2E

    xt = A_x.reshape(S, D).T
    w2t = B_w2.T
    b1 = B_b1.reshape(1, F)

    def kernel(xt_ref, wqkv_ref, wo_ref, b1_ref, w1_hbm, w2t_hbm, out_ref,
               x_s, q_s, kt_s, v_s, oacc_s, oprev_s, w1_s, w2t_s, sems):
        i = pl.program_id(0)

        @pl.when(i == 0)
        def _():
            pltpu.make_async_copy(w1_hbm, w1_s, sems.at[0]).start()
            pltpu.make_async_copy(w2t_hbm, w2t_s, sems.at[1]).start()
            lane = jax.lax.broadcasted_iota(jnp.int32, (RC, _LANES), 1)

            def piece(qkv, base, g):
                w = gw[g]
                p = qkv[:, base + g * _HPG * dh: base + g * _HPG * dh + w]
                return jnp.concatenate(
                    [p, jnp.zeros((RC, _LANES - w), jnp.float32)], axis=1)

            for c in range(S // RC):
                rows = pl.ds(c * RC, RC)
                xf = xt_ref[:, rows].astype(jnp.float32).T
                x_s[rows, :] = xf
                xn = _layernorm(xf).astype(jnp.bfloat16)
                qkv = jnp.dot(xn, wqkv_ref[...], preferred_element_type=jnp.float32)
                for g in range(ng):
                    q_s[g, rows, :] = (piece(qkv, 0, g) * scale).astype(jnp.bfloat16)
                    kt_s[g, :, rows] = piece(qkv, D, g).T.astype(jnp.bfloat16)
                    vg = jnp.where(lane == _LANES - 1, 1.0, piece(qkv, 2 * D, g))
                    v_s[g, rows, :] = vg.astype(jnp.bfloat16)

        qrows = pl.ds(pl.multiple_of(i * TQ, TQ), TQ)
        lane_q = jax.lax.broadcasted_iota(jnp.int32, (TQ, _LANES), 1)
        oacc_s[...] = jnp.zeros_like(oacc_s)

        def head_mask(h):
            g = h // _HPG
            lo = (h - g * _HPG) * dh
            return g, jnp.logical_and(lane_q >= lo, lane_q < lo + dh)

        def finalize(h):
            g, mask = head_mask(h)
            o = oprev_s[...]
            o = o / o[:, _LANES - 1:_LANES]
            oacc_s[g] = jnp.where(mask, o, oacc_s[g])

        def head_body(h, carry):
            g, mask = head_mask(h)
            qg = q_s[g, qrows, :]
            qh = jnp.where(mask, qg, jnp.zeros_like(qg))
            s = jnp.dot(qh, kt_s[g], preferred_element_type=jnp.float32)
            finalize(jnp.maximum(h - 1, 0))
            m = jnp.max(s, axis=1, keepdims=True)
            p = jnp.exp2(s - m).astype(jnp.bfloat16)
            oprev_s[...] = jnp.dot(p, v_s[g], preferred_element_type=jnp.float32)
            return carry

        oprev_s[...] = jnp.ones_like(oprev_s)
        jax.lax.fori_loop(0, _H, head_body, 0, unroll=1)
        finalize(_H - 1)

        o_all = jnp.concatenate(
            [oacc_s[g][:, :gw[g]] for g in range(ng)], axis=1).astype(jnp.bfloat16)
        attn = jnp.dot(o_all, wo_ref[...], preferred_element_type=jnp.float32)
        hres = x_s[qrows, :] + attn

        @pl.when(i == 0)
        def _():
            pltpu.make_async_copy(w1_hbm, w1_s, sems.at[0]).wait()
            pltpu.make_async_copy(w2t_hbm, w2t_s, sems.at[1]).wait()

        hn = _layernorm(hres).astype(jnp.bfloat16)
        u = jnp.dot(hn, w1_s[...], preferred_element_type=jnp.float32) + b1_ref[...].astype(jnp.float32)
        sp = jnp.log1p(jnp.exp(-jnp.abs(u))) + jnp.maximum(u, 0.0)
        act = (u * jnp.tanh(sp)).astype(jnp.bfloat16)
        y = jax.lax.dot_general(act, w2t_s[...], (((1,), (1,)), ((), ())),
                                preferred_element_type=jnp.float32)
        out_ref[...] = (hres + y).T.astype(out_ref.dtype)

    out_t = pl.pallas_call(
        kernel,
        grid=(NQ,),
        in_specs=[
            pl.BlockSpec((D, S), lambda i: (0, 0)),
            pl.BlockSpec((D, 3 * D), lambda i: (0, 0)),
            pl.BlockSpec((D, D), lambda i: (0, 0)),
            pl.BlockSpec((1, F), lambda i: (0, 0)),
            pl.BlockSpec(memory_space=pl.ANY),
            pl.BlockSpec(memory_space=pl.ANY),
        ],
        out_specs=pl.BlockSpec((D, TQ), lambda i: (0, i)),
        out_shape=jax.ShapeDtypeStruct((D, S), A_x.dtype),
        scratch_shapes=[
            pltpu.VMEM((S, D), jnp.float32),
            pltpu.VMEM((ng, S, _LANES), jnp.bfloat16),
            pltpu.VMEM((ng, _LANES, S), jnp.bfloat16),
            pltpu.VMEM((ng, S, _LANES), jnp.bfloat16),
            pltpu.VMEM((ng, TQ, _LANES), jnp.float32),
            pltpu.VMEM((TQ, _LANES), jnp.float32),
            pltpu.VMEM((D, F), jnp.bfloat16),
            pltpu.VMEM((D, F), jnp.bfloat16),
            pltpu.SemaphoreType.DMA((2,)),
        ],
        compiler_params=pltpu.CompilerParams(
            dimension_semantics=("arbitrary",),
            vmem_limit_bytes=100 * 1024 * 1024,
        ),
    )(xt, A_wqkv, A_wo, b1, B_w1, w2t)
    return out_t.T.reshape(B, S, D)
```

```python
import jax
import jax.numpy as jnp
import jax.experimental.pallas as pl
import jax.experimental.pallas.tpu as pltpu

_H = 32
_HPG = 6
_LANES = 128
_EPS = 1e-5
_LOG2E = 1.4426950408889634


def _layernorm(x):
    m = jnp.mean(x, axis=-1, keepdims=True)
    xc = x - m
    v = jnp.mean(xc * xc, axis=-1, keepdims=True)
    return xc * jax.lax.rsqrt(v + _EPS)


@jax.jit
def pallas_sequential_preLN__mha_block__dense_activation_mish__prompt_kernel(
    A_x: jax.Array,
    A_wqkv: jax.Array,
    A_wo: jax.Array,
    B_x: jax.Array,
    B_w1: jax.Array,
    B_b1: jax.Array,
    B_w2: jax.Array,
):
    B, S, D = A_x.shape
    assert B == 1
    F = B_w1.shape[1]
    dh = D // _H
    ng = -(-_H // _HPG)
    nh = [min(_HPG, _H - g * _HPG) for g in range(ng)]
    gw = [n * dh for n in nh]
    SL = _HPG * dh
    assert SL + _HPG <= _LANES
    TQ = 2048
    TM = 256
    NQ = S // TQ
    RC = 512
    scale = (dh ** -0.5) * _LOG2E

    xt = A_x.reshape(S, D).T
    w2t = B_w2.T
    b1 = B_b1.reshape(1, F)

    def kernel(xt_ref, wqkv_ref, wo_ref, b1_ref, w1_hbm, w2t_hbm, out_ref,
               x_s, q_s, kt_s, v_s, oacc_s, oa_s, w1_s, w2t_s, sems):
        i = pl.program_id(0)

        @pl.when(i == 0)
        def _():
            pltpu.make_async_copy(w1_hbm, w1_s, sems.at[0]).start()
            pltpu.make_async_copy(w2t_hbm, w2t_s, sems.at[1]).start()
            lane = jax.lax.broadcasted_iota(jnp.int32, (RC, _LANES), 1)

            def piece(qkv, base, g):
                w = gw[g]
                p = qkv[:, base + g * SL: base + g * SL + w]
                return jnp.concatenate(
                    [p, jnp.zeros((RC, _LANES - w), jnp.float32)], axis=1)

            for c in range(S // RC):
                rows = pl.ds(c * RC, RC)
                xf = xt_ref[:, rows].astype(jnp.float32).T
                x_s[rows, :] = xf
                xn = _layernorm(xf).astype(jnp.bfloat16)
                qkv = jnp.dot(xn, wqkv_ref[...], preferred_element_type=jnp.float32)
                for g in range(ng):
                    q_s[g, rows, :] = (piece(qkv, 0, g) * scale).astype(jnp.bfloat16)
                    kt_s[g, :, rows] = piece(qkv, D, g).T.astype(jnp.bfloat16)
                    vg = jnp.where(lane >= SL, 1.0, piece(qkv, 2 * D, g))
                    v_s[g, rows, :] = vg.astype(jnp.bfloat16)

        qrows = pl.ds(pl.multiple_of(i * TQ, TQ), TQ)
        lane_q = jax.lax.broadcasted_iota(jnp.int32, (TQ, _LANES), 1)
        oacc_s[...] = jnp.ones_like(oacc_s)

        def head_body(h, carry):
            g = h // _HPG
            j = h - g * _HPG
            lo = j * dh
            mask = jnp.logical_and(lane_q >= lo, lane_q < lo + dh)
            qg = q_s[g, qrows, :]
            qh = jnp.where(mask, qg, jnp.zeros_like(qg))
            s = jnp.dot(qh, kt_s[g], preferred_element_type=jnp.float32)
            m = jnp.max(s, axis=1, keepdims=True)
            p = jnp.exp2(s - m).astype(jnp.bfloat16)
            o = jnp.dot(p, v_s[g], preferred_element_type=jnp.float32)
            keep = jnp.logical_or(mask, lane_q == SL + j)
            oacc_s[g] = jnp.where(keep, o, oacc_s[g])
            return carry

        jax.lax.fori_loop(0, _H, head_body, 0)

        @pl.when(i == 0)
        def _():
            pltpu.make_async_copy(w1_hbm, w1_s, sems.at[0]).wait()
            pltpu.make_async_copy(w2t_hbm, w2t_s, sems.at[1]).wait()

        lane_m = jax.lax.broadcasted_iota(jnp.int32, (TM, _LANES), 1)

        def norm_block(jb):
            r = pl.ds(pl.multiple_of(jb * TM, TM), TM)
            pieces = []
            for g in range(ng):
                og = oacc_s[g, r, :]
                den = jnp.ones_like(og)
                for j in range(nh[g]):
                    lj = og[:, SL + j:SL + j + 1]
                    den = jnp.where(
                        jnp.logical_and(lane_m >= j * dh, lane_m < (j + 1) * dh), lj, den)
                pieces.append((og / den)[:, :gw[g]])
            return jnp.concatenate(pieces, axis=1).astype(jnp.bfloat16)

        nb = TQ // TM
        oa_s[...] = norm_block(0)

        def tail_body(jb, carry):
            r = pl.ds(pl.multiple_of(jb * TM, TM), TM)
            xr = pl.ds(pl.multiple_of(i * TQ + jb * TM, TM), TM)
            attn = jnp.dot(oa_s[...], wo_ref[...], preferred_element_type=jnp.float32)
            oa_s[...] = norm_block(jnp.minimum(jb + 1, nb - 1))
            hres = x_s[xr, :] + attn
            hn = _layernorm(hres).astype(jnp.bfloat16)
            u = jnp.dot(hn, w1_s[...], preferred_element_type=jnp.float32) + b1_ref[...].astype(jnp.float32)
            sp = jnp.log1p(jnp.exp(-jnp.abs(u))) + jnp.maximum(u, 0.0)
            act = (u * jnp.tanh(sp)).astype(jnp.bfloat16)
            y = jax.lax.dot_general(act, w2t_s[...], (((1,), (1,)), ((), ())),
                                    preferred_element_type=jnp.float32)
            out_ref[:, r] = (hres + y).T.astype(out_ref.dtype)
            return carry

        jax.lax.fori_loop(0, nb, tail_body, 0)

    out_t = pl.pallas_call(
        kernel,
        grid=(NQ,),
        in_specs=[
            pl.BlockSpec((D, S), lambda i: (0, 0)),
            pl.BlockSpec((D, 3 * D), lambda i: (0, 0)),
            pl.BlockSpec((D, D), lambda i: (0, 0)),
            pl.BlockSpec((1, F), lambda i: (0, 0)),
            pl.BlockSpec(memory_space=pl.ANY),
            pl.BlockSpec(memory_space=pl.ANY),
        ],
        out_specs=pl.BlockSpec((D, TQ), lambda i: (0, i)),
        out_shape=jax.ShapeDtypeStruct((D, S), A_x.dtype),
        scratch_shapes=[
            pltpu.VMEM((S, D), jnp.float32),
            pltpu.VMEM((ng, S, _LANES), jnp.bfloat16),
            pltpu.VMEM((ng, _LANES, S), jnp.bfloat16),
            pltpu.VMEM((ng, S, _LANES), jnp.bfloat16),
            pltpu.VMEM((ng, TQ, _LANES), jnp.float32),
            pltpu.VMEM((TM, D), jnp.bfloat16),
            pltpu.VMEM((D, F), jnp.bfloat16),
            pltpu.VMEM((D, F), jnp.bfloat16),
            pltpu.SemaphoreType.DMA((2,)),
        ],
        compiler_params=pltpu.CompilerParams(
            dimension_semantics=("arbitrary",),
            vmem_limit_bytes=100 * 1024 * 1024,
        ),
    )(xt, A_wqkv, A_wo, b1, B_w1, w2t)
    return out_t.T.reshape(B, S, D)
```
